```python
import jax
import jax.numpy as jnp

def _softmax(x, axis=-1):
    return jax.nn.softmax(x, axis=axis)

def _gelu(x):
    return jax.nn.gelu(x, approximate=True)

def _silu(x):
    return jax.nn.silu(x)

def _sigmoid(x):
    return jax.nn.sigmoid(x)

def _layernorm(x, axis=-1, eps=1e-05):
    m = jnp.mean(x, axis=axis, keepdims=True)
    v = jnp.var(x, axis=axis, keepdims=True)
    return (x - m) / jnp.sqrt(v + eps)

def _scatter_add(tgt, idx, src, axis=0):
    return tgt.at[idx].add(src)

def _segment_sum(src, seg, n):
    return jax.ops.segment_sum(src, seg, n)

class _Rng:

    def __init__(self, key):
        self._k = key

    def _next(self):
        self._k, sub = jax.random.split(self._k)
        return sub

    def normal(self, shape):
        return jax.random.normal(self._next(), shape, dtype=jnp.bfloat16)

    def randint(self, lo, hi, shape):
        return jax.random.randint(self._next(), shape, lo, hi, dtype=jnp.int32)

    def uniform(self, shape, lo=0.0, hi=1.0):
        return jax.random.uniform(self._next(), shape, jnp.bfloat16, lo, hi)

    def permutation(self, n):
        return jax.random.permutation(self._next(), n)
kernel_name = 'adaLN_cond__compressed_kv_cla__dense_activation_relu__decode'

def setup_inputs():
    _rng = _Rng(jax.random.key(int.from_bytes(__import__("os").urandom(4), "little")))
    _w = lambda a: (lambda t: t.astype(jnp.bfloat16) if jnp.issubdtype(t.dtype, jnp.floating) else t)(jnp.asarray(a))

    def _A_setup():
        B, H, Sq, Sk, D, M = (8, 32, 1, 4096, 128, 512)
        Dc = 4 * D
        return {'x': _w((lambda *s: _rng.normal(s) * 0.05)(B, Sq, M)), 'c_kv': _w((lambda *s: _rng.normal(s) * 0.05)(B, Sk, Dc)), 'w_q': _w((lambda *s: _rng.normal(s) * 0.05)(M, H, D) * M ** (-0.5)), 'w_uk': _w((lambda *s: _rng.normal(s) * 0.05)(Dc, H, D) * Dc ** (-0.5)), 'w_uv': _w((lambda *s: _rng.normal(s) * 0.05)(Dc, H, D) * Dc ** (-0.5)), 'w_o': _w((lambda *s: _rng.normal(s) * 0.05)(H, D, M) * (H * D) ** (-0.5))}
    _A_in = _A_setup()

    def _B_setup():
        B, S, D, Dff = (8, 1, 512, 1792)
        return {'x': _w((lambda *s: _rng.normal(s) * 0.05)(B, S, D)), 'w1': _w((lambda *s: _rng.normal(s) * 0.05)(D, Dff)), 'w2': _w((lambda *s: _rng.normal(s) * 0.05)(Dff, D))}
    _B_in = _B_setup()
    return {'A_x': _A_in['x'], 'A_c_kv': _A_in['c_kv'], 'A_w_q': _A_in['w_q'], 'A_w_uk': _A_in['w_uk'], 'A_w_uv': _A_in['w_uv'], 'A_w_o': _A_in['w_o'], 'B_x': _B_in['x'], 'B_w1': _B_in['w1'], 'B_w2': _B_in['w2'], 'c': _w((lambda *s: _rng.normal(s) * 0.05)(8, 512)), 'w_mod': _w((lambda *s: _rng.normal(s) * 0.05)(512, 6 * 512) * 512 ** (-0.5))}

def reference(A_x, A_c_kv, A_w_q, A_w_uk, A_w_uv, A_w_o, B_x, B_w1, B_w2, c, w_mod):

    def _A_ref(x, c_kv, w_q, w_uk, w_uv, w_o):
        B, Sq, M = (x.shape[0], x.shape[1], x.shape[2])
        Sk = c_kv.shape[1]
        H, D = (w_q.shape[1], w_q.shape[2])
        q = jnp.einsum('bqm,mhd->bhqd', x, w_q)
        k = jnp.einsum('bkc,chd->bhkd', c_kv, w_uk)
        v = jnp.einsum('bkc,chd->bhkd', c_kv, w_uv)
        scores = jnp.einsum('bhqd,bhkd->bhqk', q, k) * D ** (-0.5)
        off = Sk - Sq
        qi = jnp.arange(Sq)[:, None]
        kj = jnp.arange(Sk)[None, :]
        cmask = kj <= qi + off
        scores = jnp.where(cmask[None, None], scores, -1000000000.0)
        p = _softmax(scores, axis=-1)
        ctx = jnp.einsum('bhqk,bhkd->bhqd', p, v)
        return jnp.einsum('bhqd,hdm->bqm', ctx, w_o)

    def _B_ref(x, w1, w2):
        h = jnp.einsum('bsd,df->bsf', x, w1)
        zero = jnp.zeros_like(h)
        h = jnp.maximum(h, zero)
        return jnp.einsum('bsf,fd->bsd', h, w2)
    x = A_x
    mod = (_silu(c) @ w_mod).reshape(c.shape[0], 6, 1, -1)
    sa, ca, ga, sb, cb, gb = (mod[:, 0].copy(), mod[:, 1].copy(), mod[:, 2].copy(), mod[:, 3].copy(), mod[:, 4].copy(), mod[:, 5].copy())
    h = _layernorm(x, axis=-1) * (1 + ca) + sa
    x = x + ga * _A_ref(h, A_c_kv, A_w_q, A_w_uk, A_w_uv, A_w_o)
    h = _layernorm(x, axis=-1) * (1 + cb) + sb
    x = x + gb * _B_ref(h, B_w1, B_w2)
    return x
```

```python
import jax
import jax.numpy as jnp
from jax import lax
import jax.experimental.pallas as pl
import jax.experimental.pallas.tpu as pltpu

F32, BF16, U32 = jnp.float32, jnp.bfloat16, jnp.uint32
_NT = (((1,), (1,)), ((), ()))
_LANES = 128
_WINDOW = 3


def _layernorm(x):
    d = x - jnp.mean(x, axis=-1, keepdims=True)
    v = jnp.mean(d * d, axis=-1, keepdims=True)
    return d / jnp.sqrt(v + 1e-5)


def _head_pair(w_ref, j, rows, n_pairs):
    w = w_ref[pl.ds(j, rows, stride=n_pairs), :]
    lo = pltpu.bitcast(w << 16, F32).astype(BF16)
    hi = pltpu.bitcast(w & jnp.uint32(0xFFFF0000), F32).astype(BF16)
    return lo, hi


@jax.jit
def pallas_adaLN_cond__compressed_kv_cla__dense_activation_relu__decode_kernel(
    A_x: jax.Array,
    A_c_kv: jax.Array,
    A_w_q: jax.Array,
    A_w_uk: jax.Array,
    A_w_uv: jax.Array,
    A_w_o: jax.Array,
    B_x: jax.Array,
    B_w1: jax.Array,
    B_w2: jax.Array,
    c: jax.Array,
    w_mod: jax.Array,
):
    del B_x
    B, Sq, M = A_x.shape
    _, _, Dc = A_c_kv.shape
    _, H, D = A_w_q.shape
    assert Sq == 1 and D == _LANES and H % 2 == 0 and Dc % _LANES == 0
    n_pairs, c_tiles = H // 2, Dc // _LANES

    order = (["mod_a", "w_q", "w_uk"] + [f"kv{b}" for b in range(B)]
             + ["w_uv", "w_o", "w1", "w2", "mod_b"])
    names = ["x", "c"] + order

    def kernel(x_h, c_h, wmod_h, wq_h, wuk_h, ckv_h, wuv_h, wo_h, w1_h, w2_h, o_ref,
               x_v, c_v, wmod_v, wq_v, wuk_v, ckv_v, wuv_v, wo_v, w1_v, w2_v,
               head_s, qlat_s, clat_s, sems):
        def mod_cols(first, n):
            cols = pl.ds(first * M, n * M)
            return wmod_h.at[:, cols], wmod_v.at[:, cols]

        ends = dict(
            x=(x_h, x_v), c=(c_h, c_v), mod_a=mod_cols(0, 5), mod_b=mod_cols(5, 1),
            w_q=(wq_h.bitcast(U32), wq_v), w_uk=(wuk_h.bitcast(U32), wuk_v),
            w_uv=(wuv_h.bitcast(U32), wuv_v), w_o=(wo_h, wo_v),
            w1=(w1_h, w1_v), w2=(w2_h, w2_v),
            **{f"kv{b}": (ckv_h.at[b], ckv_v.at[b]) for b in range(B)})

        def dma(name):
            return pltpu.make_async_copy(*ends[name], sems.at[names.index(name)])

        def arrive(name):
            dma(name).wait()
            nxt = order.index(name) + _WINDOW
            if nxt < len(order):
                dma(order[nxt]).start()

        for name in [order[0], "x", "c"] + order[1:_WINDOW]:
            dma(name).start()

        dma("x").wait()
        dma("c").wait()
        cond = c_v[...].astype(F32)
        cond = (cond * jax.nn.sigmoid(cond)).astype(BF16)
        x = x_v[...].astype(F32)
        arrive("mod_a")
        mod = jnp.dot(cond, wmod_v[:, :5 * M], preferred_element_type=F32)
        sa, ca, ga, sb, cb = (mod[:, i * M:(i + 1) * M] for i in range(5))
        h = (_layernorm(x) * (1.0 + ca) + sa).astype(BF16)

        arrive("w_q")

        def q_step(j, carry):
            for i, w in enumerate(_head_pair(wq_v, j, M, n_pairs)):
                head_s[2 * j + i] = jnp.dot(h, w, preferred_element_type=F32)
            return carry

        lax.fori_loop(0, n_pairs, q_step, 0)
        arrive("w_uk")

        def absorb_k_step(j, carry):
            for i, w in enumerate(_head_pair(wuk_v, j, Dc, n_pairs)):
                q_lat = lax.dot_general(head_s[2 * j + i].astype(BF16), w, _NT,
                                        preferred_element_type=F32)
                rows = pl.ds(pl.multiple_of((2 * j + i) * B, B), B)
                for t in range(c_tiles):
                    qlat_s[t, rows, :] = q_lat[:, t * _LANES:(t + 1) * _LANES]
            return carry

        lax.fori_loop(0, n_pairs, absorb_k_step, 0)

        def attend_step(b, carry):
            for i in range(B):
                pl.when(b == i)(lambda i=i: arrive(f"kv{i}"))
            q_lat = jnp.concatenate(
                [qlat_s[t, pl.ds(b, H, stride=B), :] for t in range(c_tiles)],
                axis=1).astype(BF16)
            s = lax.dot_general(q_lat, ckv_v[b], _NT,
                                preferred_element_type=F32) * (D ** -0.5)
            p = jnp.exp(s - jnp.max(s, axis=-1, keepdims=True))
            denom = jnp.sum(p, axis=-1, keepdims=True)
            c_lat = jnp.dot(p.astype(BF16), ckv_v[b], preferred_element_type=F32) / denom
            rows = pl.ds(pl.multiple_of(b * H, H), H)
            for t in range(c_tiles):
                clat_s[t, rows, :] = c_lat[:, t * _LANES:(t + 1) * _LANES]
            return carry

        lax.fori_loop(0, B, attend_step, 0)

        arrive("w_uv")

        def absorb_v_step(j, carry):
            for i, w in enumerate(_head_pair(wuv_v, j, Dc, n_pairs)):
                c_lat = jnp.concatenate(
                    [clat_s[t, pl.ds(2 * j + i, B, stride=H), :] for t in range(c_tiles)],
                    axis=1).astype(BF16)
                head_s[2 * j + i] = jnp.dot(c_lat, w, preferred_element_type=F32)
            return carry

        lax.fori_loop(0, n_pairs, absorb_v_step, 0)
        arrive("w_o")
        ctx = jnp.concatenate([head_s[i] for i in range(H)], axis=1).astype(BF16)
        x = x + ga * jnp.dot(ctx, wo_v[...], preferred_element_type=F32)

        h = (_layernorm(x) * (1.0 + cb) + sb).astype(BF16)
        arrive("w1")
        f = jnp.maximum(jnp.dot(h, w1_v[...], preferred_element_type=F32), 0.0)
        arrive("w2")
        y = jnp.dot(f.astype(BF16), w2_v[...], preferred_element_type=F32)
        arrive("mod_b")
        gb = jnp.dot(cond, wmod_v[:, 5 * M:], preferred_element_type=F32)
        o_ref[...] = (x + gb * y).astype(o_ref.dtype)

    operands = [
        A_x.reshape(B, M), c, w_mod, A_w_q.reshape(M * H, D), A_w_uk.reshape(Dc * H, D),
        A_c_kv, A_w_uv.reshape(Dc * H, D), A_w_o.reshape(H * D, M), B_w1, B_w2,
    ]
    per_head = (3, 4, 6)
    landing = [
        pltpu.VMEM((a.shape[0] // 2, D), U32) if i in per_head else pltpu.VMEM(a.shape, a.dtype)
        for i, a in enumerate(operands)
    ]
    out = pl.pallas_call(
        kernel,
        out_shape=jax.ShapeDtypeStruct((B, M), A_x.dtype),
        in_specs=[pl.BlockSpec(memory_space=pl.ANY)] * len(operands),
        scratch_shapes=landing + [
            pltpu.VMEM((H, B, D), F32),
            pltpu.VMEM((c_tiles, H * B, _LANES), F32),
            pltpu.VMEM((c_tiles, B * H, _LANES), F32),
            pltpu.SemaphoreType.DMA((len(names),)),
        ],
        compiler_params=pltpu.CompilerParams(vmem_limit_bytes=100 * 2**20),
    )(*operands)
    return out.reshape(A_x.shape)
```

```python
import jax
import jax.numpy as jnp
from jax import lax
import jax.experimental.pallas as pl
import jax.experimental.pallas.tpu as pltpu

F32, BF16, U32 = jnp.float32, jnp.bfloat16, jnp.uint32
_NT = (((1,), (1,)), ((), ()))
_LANES = 128
_WINDOW = 4
_W2_TAIL = (384, 256, 128)
_REPACK_ROWS = 1024


def _layernorm(x):
    d = x - jnp.mean(x, axis=-1, keepdims=True)
    v = jnp.mean(d * d, axis=-1, keepdims=True)
    return d / jnp.sqrt(v + 1e-5)


def _to_words(w_ref, words_ref):
    def step(i, carry):
        src = pl.ds(pl.multiple_of(i * _REPACK_ROWS, _REPACK_ROWS), _REPACK_ROWS)
        half = _REPACK_ROWS // 2
        words_ref[pl.ds(pl.multiple_of(i * half, half), half), :] = pltpu.bitcast(
            w_ref[src, :], U32)
        return carry

    lax.fori_loop(0, w_ref.shape[0] // _REPACK_ROWS, step, 0)


def _head_pair(words_ref, j, rows, n_pairs):
    w = words_ref[pl.ds(j, rows, stride=n_pairs), :]
    lo = pltpu.bitcast(w << 16, F32).astype(BF16)
    hi = pltpu.bitcast(w & jnp.uint32(0xFFFF0000), F32).astype(BF16)
    return lo, hi


@jax.jit
def pallas_adaLN_cond__compressed_kv_cla__dense_activation_relu__decode_kernel(
    A_x: jax.Array,
    A_c_kv: jax.Array,
    A_w_q: jax.Array,
    A_w_uk: jax.Array,
    A_w_uv: jax.Array,
    A_w_o: jax.Array,
    B_x: jax.Array,
    B_w1: jax.Array,
    B_w2: jax.Array,
    c: jax.Array,
    w_mod: jax.Array,
):
    del B_x
    B, Sq, M = A_x.shape
    _, _, Dc = A_c_kv.shape
    _, H, D = A_w_q.shape
    assert Sq == 1
    assert D == _LANES and H % 2 == 0 and Dc % _LANES == 0
    assert A_w_q.dtype == A_w_uk.dtype == A_w_uv.dtype == BF16
    assert (M * H) % _REPACK_ROWS == 0 and (Dc * H) % _REPACK_ROWS == 0
    n_pairs, c_tiles = H // 2, Dc // _LANES

    w2_sizes = (B_w2.shape[0] - sum(_W2_TAIL),) + _W2_TAIL
    w2_blocks = [pl.ds(sum(w2_sizes[:i]), n) for i, n in enumerate(w2_sizes)]
    order = (["w_mod", "w_q", "w_uk"] + [f"kv{b}" for b in range(B)]
             + ["w_uv", "w_o", "w1"] + [f"w2_{i}" for i in range(len(w2_blocks))])
    names = ["x", "c"] + order

    def body(x_h, c_h, wmod_h, wq_h, wuk_h, ckv_h, wuv_h, wo_h, w1_h, w2_h, o_ref,
             x_v, c_v, wmod_v, wq_v, wuk_v, ckv_v, wuv_v, wo_v, w1_v, w2_v,
             words_s, head_s, qlat_s, clat_s, sems):
        ends = dict(
            x=(x_h, x_v), c=(c_h, c_v), w_mod=(wmod_h, wmod_v), w_q=(wq_h, wq_v),
            w_uk=(wuk_h, wuk_v), w_uv=(wuv_h, wuv_v), w_o=(wo_h, wo_v), w1=(w1_h, w1_v),
            **{f"kv{b}": (ckv_h.at[b], ckv_v.at[b]) for b in range(B)},
            **{f"w2_{i}": (w2_h.at[r], w2_v.at[r]) for i, r in enumerate(w2_blocks)})

        def dma(name):
            return pltpu.make_async_copy(*ends[name], sems.at[names.index(name)])

        def arrive(name):
            dma(name).wait()
            nxt = order.index(name) + _WINDOW
            if nxt < len(order):
                dma(order[nxt]).start()

        for name in [order[0], "x", "c"] + order[1:_WINDOW]:
            dma(name).start()

        dma("x").wait()
        dma("c").wait()
        cond = c_v[...].astype(F32)
        cond = (cond * jax.nn.sigmoid(cond)).astype(BF16)
        x = x_v[...].astype(F32)
        arrive("w_mod")
        mod = jnp.dot(cond, wmod_v[...], preferred_element_type=F32)
        sa, ca, ga, sb, cb, gb = (mod[:, i * M:(i + 1) * M] for i in range(6))
        h = (_layernorm(x) * (1.0 + ca) + sa).astype(BF16)

        arrive("w_q")
        _to_words(wq_v, words_s)

        def q_step(j, carry):
            for i, w in enumerate(_head_pair(words_s, j, M, n_pairs)):
                head_s[2 * j + i] = jnp.dot(h, w, preferred_element_type=F32)
            return carry

        lax.fori_loop(0, n_pairs, q_step, 0)
        arrive("w_uk")
        _to_words(wuk_v, words_s)

        def absorb_k_step(j, carry):
            for i, w in enumerate(_head_pair(words_s, j, Dc, n_pairs)):
                q_lat = lax.dot_general(head_s[2 * j + i].astype(BF16), w, _NT,
                                        preferred_element_type=F32)
                rows = pl.ds(pl.multiple_of((2 * j + i) * B, B), B)
                for t in range(c_tiles):
                    qlat_s[t, rows, :] = q_lat[:, t * _LANES:(t + 1) * _LANES]
            return carry

        lax.fori_loop(0, n_pairs, absorb_k_step, 0)

        def attend_step(b, carry):
            for i in range(B):
                pl.when(b == i)(lambda i=i: arrive(f"kv{i}"))
            q_lat = jnp.concatenate(
                [qlat_s[t, pl.ds(b, H, stride=B), :] for t in range(c_tiles)],
                axis=1).astype(BF16)
            s = lax.dot_general(q_lat, ckv_v[b], _NT,
                                preferred_element_type=F32) * (D ** -0.5)
            p = jnp.exp(s - jnp.max(s, axis=-1, keepdims=True))
            denom = jnp.sum(p, axis=-1, keepdims=True)
            c_lat = jnp.dot(p.astype(BF16), ckv_v[b], preferred_element_type=F32) / denom
            rows = pl.ds(pl.multiple_of(b * H, H), H)
            for t in range(c_tiles):
                clat_s[t, rows, :] = c_lat[:, t * _LANES:(t + 1) * _LANES]
            return carry

        lax.fori_loop(0, B, attend_step, 0)

        arrive("w_uv")
        _to_words(wuv_v, words_s)

        def absorb_v_step(j, carry):
            for i, w in enumerate(_head_pair(words_s, j, Dc, n_pairs)):
                c_lat = jnp.concatenate(
                    [clat_s[t, pl.ds(2 * j + i, B, stride=H), :] for t in range(c_tiles)],
                    axis=1).astype(BF16)
                head_s[2 * j + i] = jnp.dot(c_lat, w, preferred_element_type=F32)
            return carry

        lax.fori_loop(0, n_pairs, absorb_v_step, 0)
        arrive("w_o")
        ctx = jnp.concatenate([head_s[i] for i in range(H)], axis=1).astype(BF16)
        x = x + ga * jnp.dot(ctx, wo_v[...], preferred_element_type=F32)

        h = (_layernorm(x) * (1.0 + cb) + sb).astype(BF16)
        arrive("w1")
        f = jnp.maximum(jnp.dot(h, w1_v[...], preferred_element_type=F32), 0.0).astype(BF16)
        for i, r in enumerate(w2_blocks):
            arrive(f"w2_{i}")
            x = x + gb * jnp.dot(f[:, r.start:r.start + r.size], w2_v[r, :],
                                 preferred_element_type=F32)
        o_ref[...] = x.astype(o_ref.dtype)

    def kernel(*refs):
        pl.run_scoped(lambda sems: body(*refs, sems),
                      pltpu.SemaphoreType.DMA((len(names),)))

    operands = [
        A_x.reshape(B, M), c, w_mod, A_w_q.reshape(M * H, D), A_w_uk.reshape(Dc * H, D),
        A_c_kv, A_w_uv.reshape(Dc * H, D), A_w_o.reshape(H * D, M), B_w1, B_w2,
    ]
    out = pl.pallas_call(
        kernel,
        out_shape=jax.ShapeDtypeStruct((B, M), A_x.dtype),
        in_specs=[pl.BlockSpec(memory_space=pl.ANY)] * len(operands),
        scratch_shapes=[pltpu.VMEM(a.shape, a.dtype) for a in operands] + [
            pltpu.VMEM((max(M, Dc) * n_pairs, D), U32),
            pltpu.VMEM((H, B, D), F32),
            pltpu.VMEM((c_tiles, H * B, _LANES), F32),
            pltpu.VMEM((c_tiles, B * H, _LANES), F32),
        ],
        compiler_params=pltpu.CompilerParams(vmem_limit_bytes=100 * 2**20),
    )(*operands)
    return out.reshape(A_x.shape)
```

```python
import jax
import jax.numpy as jnp
from jax import lax
import jax.experimental.pallas as pl
import jax.experimental.pallas.tpu as pltpu

F32, BF16, U32 = jnp.float32, jnp.bfloat16, jnp.uint32
_NT = (((1,), (1,)), ((), ()))
_LANES = 128
_ROW_TILE = 8
_URGENT_SHARE = 5 / 16
_W2_TAIL = (384, 256, 128)


def _layernorm(x):
    d = x - jnp.mean(x, axis=-1, keepdims=True)
    v = jnp.mean(d * d, axis=-1, keepdims=True)
    return d / jnp.sqrt(v + 1e-5)


def _block(i, n, offset=0, size=None):
    start = i * n + offset
    if not isinstance(start, int):
        start = pl.multiple_of(start, _ROW_TILE if offset else n)
    return pl.ds(start, n if size is None else size)


def _lane_tiles(a):
    return [a[:, u:u + _LANES] for u in range(0, a.shape[1], _LANES)]


def _head_pair(words_ref, j, rows, n_pairs):
    w = words_ref[pl.ds(j, rows, stride=n_pairs), :]
    lo = pltpu.bitcast(w << 16, F32).astype(BF16)
    hi = pltpu.bitcast(w & jnp.uint32(0xFFFF0000), F32).astype(BF16)
    return lo, hi


@jax.jit
def pallas_adaLN_cond__compressed_kv_cla__dense_activation_relu__decode_kernel(
    A_x: jax.Array,
    A_c_kv: jax.Array,
    A_w_q: jax.Array,
    A_w_uk: jax.Array,
    A_w_uv: jax.Array,
    A_w_o: jax.Array,
    B_x: jax.Array,
    B_w1: jax.Array,
    B_w2: jax.Array,
    c: jax.Array,
    w_mod: jax.Array,
):
    del B_x
    B, Sq, M = A_x.shape
    _, Sk, Dc = A_c_kv.shape
    _, H, D = A_w_q.shape
    assert Sq == 1
    T = H // 2
    keys = Sk // T
    c_tiles = Dc // _LANES
    assert D == _LANES and H % 2 == 0 and Dc % _LANES == 0 and B >= 3
    assert Sk % (T * _LANES) == 0 and M % (T * 2 * _ROW_TILE) == 0
    assert A_w_q.dtype == A_w_uk.dtype == A_w_uv.dtype == BF16

    w2_sizes = (B_w2.shape[0] - sum(_W2_TAIL),) + _W2_TAIL
    w2_blocks = [pl.ds(sum(w2_sizes[:i]), n) for i, n in enumerate(w2_sizes)]

    def body(x_h, c_h, wmod_h, wq_h, wuk_h, ckv_h, wuv_h, wo_h, w1_h, w2_h, o_ref,
             x_v, c_v, wmod_v, wq_v, wuk_v, ckv_v, wuv_v, wo_v, w1_v, w2_v,
             words_a, words_b, head_s, qlat_s, q_s, score_s, clat_s,
             chunk_sems, sems):
        stream = ([(wmod_h, wmod_v), (wq_h, wq_v), (wuk_h, wuk_v)]
                  + [(ckv_h.at[b], ckv_v.at[b]) for b in range(B)]
                  + [(wuv_h, wuv_v), (wo_h, wo_v), (w1_h, w1_v)])
        W_MOD, W_Q, W_UK, KV, W_UV, W_O, W_1 = 0, 1, 2, 3, 3 + B, 4 + B, 5 + B

        def chunk_copy(s, t, offset=0, size=None):
            src, dst = stream[s]
            rows = _block(t, src.shape[0] // T, offset, size)
            return pltpu.make_async_copy(
                src.at[rows], dst.at[rows], chunk_sems.at[(s % 2) * T + t])

        def start_chunk(s, t):
            n = stream[s][0].shape[0] // T
            urgent = int(n * _URGENT_SHARE) // _ROW_TILE * _ROW_TILE
            chunk_copy(s, t, n - urgent, urgent).start(priority=0)
            chunk_copy(s, t, 0, n - urgent).start(priority=1)

        def stage(s, *jobs):
            def step(t, carries):
                chunk_copy(s, t).wait()
                if s + 1 < len(stream):
                    start_chunk(s + 1, t)
                return tuple(job(t, carry) for (job, _), carry in zip(jobs, carries))

            return lax.fori_loop(0, T, step, tuple(init for _, init in jobs))

        def to_words(w_ref, words_ref):
            n = w_ref.shape[0] // T

            def step(t, carry):
                words_ref[_block(t, n // 2), :] = pltpu.bitcast(w_ref[_block(t, n), :], U32)
                return carry

            return step, 0

        small = [pltpu.make_async_copy(x_h, x_v, sems.at[0]),
                 pltpu.make_async_copy(c_h, c_v, sems.at[1])]
        w2_copies = [pltpu.make_async_copy(w2_h.at[r], w2_v.at[r], sems.at[2 + i])
                     for i, r in enumerate(w2_blocks)]
        for t in range(T):
            start_chunk(W_MOD, t)
        for copy in small:
            copy.start()

        stage(W_MOD)
        for copy in small:
            copy.wait()
        cond = c_v[...].astype(F32)
        cond = (cond * jax.nn.sigmoid(cond)).astype(BF16)
        mod = jnp.dot(cond, wmod_v[...], preferred_element_type=F32)
        sa, ca, ga, sb, cb, gb = (mod[:, i * M:(i + 1) * M] for i in range(6))
        x = x_v[...].astype(F32)
        h = (_layernorm(x) * (1.0 + ca) + sa).astype(BF16)

        def project_q(j, carry):
            for i, w in enumerate(_head_pair(words_a, j, M, T)):
                head_s[2 * j + i] = jnp.dot(h, w, preferred_element_type=F32)
            return carry

        def absorb_k(j, carry):
            for i, w in enumerate(_head_pair(words_b, j, Dc, T)):
                q_lat = lax.dot_general(head_s[2 * j + i].astype(BF16), w, _NT,
                                        preferred_element_type=F32)
                for u, tile in enumerate(_lane_tiles(q_lat)):
                    qlat_s[u, _block(2 * j + i, B), :] = tile
            return carry

        stage(W_Q, to_words(wq_v, words_a))
        stage(W_UK, to_words(wuk_v, words_b), (project_q, 0))
        stage(KV, (absorb_k, 0))
        for b in range(B):
            q_s[b] = jnp.concatenate(
                [qlat_s[u, pl.ds(b, H, stride=B), :] for u in range(c_tiles)],
                axis=1).astype(BF16)

        def scores(b):
            def step(t, top):
                s = lax.dot_general(q_s[b], ckv_v[b, _block(t, keys), :], _NT,
                                    preferred_element_type=F32) * (D ** -0.5)
                score_s[b, t] = s
                for tile in _lane_tiles(s):
                    top = jnp.maximum(top, tile)
                return top

            return step, jnp.full((H, _LANES), -jnp.inf, F32)

        def context(b, top):
            row_max = jnp.max(top, axis=-1, keepdims=True)

            def step(t, carry):
                acc, total = carry
                p = jnp.exp(score_s[b, t] - row_max)
                acc = acc + jnp.dot(p.astype(BF16), ckv_v[b, _block(t, keys), :],
                                    preferred_element_type=F32)
                return acc, sum(_lane_tiles(p), total)

            return step, (jnp.zeros((H, Dc), F32), jnp.zeros((H, _LANES), F32))

        def normalize(b, carry):
            acc, total = carry
            c_lat = acc / jnp.sum(total, axis=-1, keepdims=True)
            for u, tile in enumerate(_lane_tiles(c_lat)):
                clat_s[u, _block(b, H), :] = tile

        top0, top1 = stage(KV + 1, scores(0), scores(1))
        top, ctx0, ctx1 = stage(KV + 2, scores(2), context(0, top0), context(1, top1))
        normalize(0, ctx0)
        normalize(1, ctx1)
        for b in range(3, B):
            top, ctx = stage(KV + b, scores(b), context(b - 1, top))
            normalize(b - 1, ctx)
        _, ctx = stage(W_UV, to_words(wuv_v, words_a), context(B - 1, top))
        normalize(B - 1, ctx)

        def absorb_v(j, carry):
            for i, w in enumerate(_head_pair(words_a, j, Dc, T)):
                c_lat = jnp.concatenate(
                    [clat_s[u, pl.ds(2 * j + i, B, stride=H), :] for u in range(c_tiles)],
                    axis=1).astype(BF16)
                head_s[2 * j + i] = jnp.dot(c_lat, w, preferred_element_type=F32)
            return carry

        stage(W_O, (absorb_v, 0))
        for copy in w2_copies:
            copy.start(priority=1)
        ctx = jnp.concatenate([head_s[i] for i in range(H)], axis=1).astype(BF16)
        x = x + ga * jnp.dot(ctx, wo_v[...], preferred_element_type=F32)

        h = (_layernorm(x) * (1.0 + cb) + sb).astype(BF16)
        stage(W_1)
        f = jnp.maximum(jnp.dot(h, w1_v[...], preferred_element_type=F32), 0.0).astype(BF16)
        for copy, r in zip(w2_copies, w2_blocks):
            copy.wait()
            x = x + gb * jnp.dot(f[:, r.start:r.start + r.size], w2_v[r, :],
                                 preferred_element_type=F32)
        o_ref[...] = x.astype(o_ref.dtype)

    def kernel(*refs):
        pl.run_scoped(lambda *sems: body(*refs, *sems),
                      pltpu.SemaphoreType.DMA((2 * T,)),
                      pltpu.SemaphoreType.DMA((2 + len(w2_blocks),)))

    operands = [
        A_x.reshape(B, M), c, w_mod, A_w_q.reshape(M * H, D), A_w_uk.reshape(Dc * H, D),
        A_c_kv, A_w_uv.reshape(Dc * H, D), A_w_o.reshape(H * D, M), B_w1, B_w2,
    ]
    out = pl.pallas_call(
        kernel,
        out_shape=jax.ShapeDtypeStruct((B, M), A_x.dtype),
        in_specs=[pl.BlockSpec(memory_space=pl.ANY)] * len(operands),
        scratch_shapes=[pltpu.VMEM(a.shape, a.dtype) for a in operands] + [
            pltpu.VMEM((max(M, Dc) * T, D), U32),
            pltpu.VMEM((Dc * T, D), U32),
            pltpu.VMEM((H, B, D), F32),
            pltpu.VMEM((c_tiles, H * B, _LANES), F32),
            pltpu.VMEM((B, H, Dc), BF16),
            pltpu.VMEM((B, T, H, keys), F32),
            pltpu.VMEM((c_tiles, B * H, _LANES), F32),
        ],
        compiler_params=pltpu.CompilerParams(vmem_limit_bytes=100 * 2**20),
    )(*operands)
    return out.reshape(A_x.shape)
```

```python
import jax
import jax.numpy as jnp
from jax import lax
import jax.experimental.pallas as pl
import jax.experimental.pallas.tpu as pltpu

F32, BF16, U32 = jnp.float32, jnp.bfloat16, jnp.uint32
_NT = (((1,), (1,)), ((), ()))
_LANES = 128
_ROW_TILE = 16
_URGENT_SHARE = 5 / 16
_W2_TAIL = (384, 256, 128)


def _layernorm(x):
    d = x - jnp.mean(x, axis=-1, keepdims=True)
    v = jnp.mean(d * d, axis=-1, keepdims=True)
    return d / jnp.sqrt(v + 1e-5)


def _block(i, n, offset=0, size=None):
    start = i * n + offset
    if not isinstance(start, int):
        start = pl.multiple_of(start, _ROW_TILE if offset else n)
    return pl.ds(start, n if size is None else size)


def _lane_tiles(a):
    return [a[:, u:u + _LANES] for u in range(0, a.shape[1], _LANES)]


def _head_pair(words_ref, j, rows, n_pairs):
    w = words_ref[pl.ds(j, rows, stride=n_pairs), :]
    lo = pltpu.bitcast(w << 16, F32).astype(BF16)
    hi = pltpu.bitcast(w & jnp.uint32(0xFFFF0000), F32).astype(BF16)
    return lo, hi


@jax.jit
def pallas_adaLN_cond__compressed_kv_cla__dense_activation_relu__decode_kernel(
    A_x: jax.Array,
    A_c_kv: jax.Array,
    A_w_q: jax.Array,
    A_w_uk: jax.Array,
    A_w_uv: jax.Array,
    A_w_o: jax.Array,
    B_x: jax.Array,
    B_w1: jax.Array,
    B_w2: jax.Array,
    c: jax.Array,
    w_mod: jax.Array,
):
    del B_x
    B, Sq, M = A_x.shape
    _, Sk, Dc = A_c_kv.shape
    _, H, D = A_w_q.shape
    assert Sq == 1
    T = H // 2
    keys = Sk // T
    c_tiles = Dc // _LANES
    assert D == _LANES and H % 2 == 0 and Dc % _LANES == 0 and B >= 3
    assert Sk % (T * _LANES) == 0 and M % (T * 2 * _ROW_TILE) == 0
    assert A_w_q.dtype == A_w_uk.dtype == A_w_uv.dtype == BF16

    w2_sizes = (B_w2.shape[0] - sum(_W2_TAIL),) + _W2_TAIL
    w2_blocks = [pl.ds(sum(w2_sizes[:i]), n) for i, n in enumerate(w2_sizes)]

    def body(x_h, c_h, wmod_h, wq_h, wuk_h, ckv_h, wuv_h, wo_h, w1_h, w2_h, o_ref,
             x_v, c_v, wmod_v, wq_v, wuk_v, ckv_v, wuv_v, wo_v, w1_v, w2_v,
             words_a, words_b, head_s, qlat_s, q_s, score_s, clat_s,
             chunk_sems, sems):
        stream = ([(wmod_h, wmod_v), (wq_h, wq_v), (wuk_h, wuk_v)]
                  + [(ckv_h.at[b], ckv_v.at[b]) for b in range(B)]
                  + [(wuv_h, wuv_v), (wo_h, wo_v), (w1_h, w1_v)])
        W_MOD, W_Q, W_UK, KV, W_UV, W_O, W_1 = 0, 1, 2, 3, 3 + B, 4 + B, 5 + B

        def chunk_copies(s, t):
            src, dst = stream[s]
            n = src.shape[0] // T
            urgent = max(1, int(n * _URGENT_SHARE) // _ROW_TILE) * _ROW_TILE
            parts = _block(t, n, n - urgent, urgent), _block(t, n, 0, n - urgent)
            sem = chunk_sems.at[(s % 2) * T + t]
            return [pltpu.make_async_copy(src.at[r], dst.at[r], sem) for r in parts]

        def start_chunk(s, t):
            for priority, copy in enumerate(chunk_copies(s, t)):
                copy.start(priority=priority)

        def stage(s, *jobs):
            def step(t, carries):
                for copy in chunk_copies(s, t):
                    copy.wait()
                if s + 1 < len(stream):
                    start_chunk(s + 1, t)
                return tuple(job(t, carry) for (job, _), carry in zip(jobs, carries))

            return lax.fori_loop(0, T, step, tuple(init for _, init in jobs))

        def to_words(w_ref, words_ref):
            n = w_ref.shape[0] // T

            def step(t, carry):
                words_ref[_block(t, n // 2), :] = pltpu.bitcast(w_ref[_block(t, n), :], U32)
                return carry

            return step, 0

        small = [pltpu.make_async_copy(x_h, x_v, sems.at[0]),
                 pltpu.make_async_copy(c_h, c_v, sems.at[1])]
        w2_copies = [pltpu.make_async_copy(w2_h.at[r], w2_v.at[r], sems.at[2 + i])
                     for i, r in enumerate(w2_blocks)]
        for t in range(T):
            start_chunk(W_MOD, t)
        for copy in small:
            copy.start()

        stage(W_MOD)
        for copy in small:
            copy.wait()
        cond = c_v[...].astype(F32)
        cond = (cond * jax.nn.sigmoid(cond)).astype(BF16)
        mod = jnp.dot(cond, wmod_v[...], preferred_element_type=F32)
        sa, ca, ga, sb, cb, gb = (mod[:, i * M:(i + 1) * M] for i in range(6))
        x = x_v[...].astype(F32)
        h = (_layernorm(x) * (1.0 + ca) + sa).astype(BF16)

        def project_q(j, carry):
            for i, w in enumerate(_head_pair(words_a, j, M, T)):
                head_s[2 * j + i] = jnp.dot(h, w, preferred_element_type=F32)
            return carry

        def absorb_k(j, carry):
            for i, w in enumerate(_head_pair(words_b, j, Dc, T)):
                q_lat = lax.dot_general(head_s[2 * j + i].astype(BF16), w, _NT,
                                        preferred_element_type=F32)
                for u, tile in enumerate(_lane_tiles(q_lat)):
                    qlat_s[u, _block(2 * j + i, B), :] = tile
            return carry

        stage(W_Q, to_words(wq_v, words_a))
        stage(W_UK, to_words(wuk_v, words_b), (project_q, 0))
        stage(KV, (absorb_k, 0))
        for b in range(B):
            q_s[b] = jnp.concatenate(
                [qlat_s[u, pl.ds(b, H, stride=B), :] for u in range(c_tiles)],
                axis=1).astype(BF16)

        def scores(b):
            def step(t, top):
                s = lax.dot_general(q_s[b], ckv_v[b, _block(t, keys), :], _NT,
                                    preferred_element_type=F32) * (D ** -0.5)
                score_s[b, t] = s
                for tile in _lane_tiles(s):
                    top = jnp.maximum(top, tile)
                return top

            return step, jnp.full((H, _LANES), -jnp.inf, F32)

        def context(b, top):
            row_max = jnp.max(top, axis=-1, keepdims=True)

            def step(t, carry):
                acc, total = carry
                p = jnp.exp(score_s[b, t] - row_max)
                acc = acc + jnp.dot(p.astype(BF16), ckv_v[b, _block(t, keys), :],
                                    preferred_element_type=F32)
                return acc, sum(_lane_tiles(p), total)

            return step, (jnp.zeros((H, Dc), F32), jnp.zeros((H, _LANES), F32))

        def normalize(b, carry):
            acc, total = carry
            c_lat = acc / jnp.sum(total, axis=-1, keepdims=True)
            for u, tile in enumerate(_lane_tiles(c_lat)):
                clat_s[u, _block(b, H), :] = tile

        top0, top1 = stage(KV + 1, scores(0), scores(1))
        top, ctx0, ctx1 = stage(KV + 2, scores(2), context(0, top0), context(1, top1))
        normalize(0, ctx0)
        normalize(1, ctx1)
        for b in range(3, B):
            top, ctx = stage(KV + b, scores(b), context(b - 1, top))
            normalize(b - 1, ctx)
        _, ctx = stage(W_UV, to_words(wuv_v, words_a), context(B - 1, top))
        normalize(B - 1, ctx)

        def absorb_v(j, carry):
            for i, w in enumerate(_head_pair(words_a, j, Dc, T)):
                c_lat = jnp.concatenate(
                    [clat_s[u, pl.ds(2 * j + i, B, stride=H), :] for u in range(c_tiles)],
                    axis=1).astype(BF16)
                head_s[2 * j + i] = jnp.dot(c_lat, w, preferred_element_type=F32)
            return carry

        stage(W_O, (absorb_v, 0))
        for copy in w2_copies:
            copy.start(priority=1)
        ctx = jnp.concatenate([head_s[i] for i in range(H)], axis=1).astype(BF16)
        x = x + ga * jnp.dot(ctx, wo_v[...], preferred_element_type=F32)

        h2 = (_layernorm(x) * (1.0 + cb) + sb).astype(BF16)
        stage(W_1)
        f = jnp.maximum(jnp.dot(h2, w1_v[...], preferred_element_type=F32), 0.0).astype(BF16)
        for copy, r in zip(w2_copies, w2_blocks):
            copy.wait()
            x = x + gb * jnp.dot(f[:, r.start:r.start + r.size], w2_v[r, :],
                                 preferred_element_type=F32)
        o_ref[...] = x.astype(o_ref.dtype)

    def kernel(*refs):
        pl.run_scoped(lambda *sems: body(*refs, *sems),
                      pltpu.SemaphoreType.DMA((2 * T,)),
                      pltpu.SemaphoreType.DMA((2 + len(w2_blocks),)))

    operands = [
        A_x.reshape(B, M), c, w_mod, A_w_q.reshape(M * H, D), A_w_uk.reshape(Dc * H, D),
        A_c_kv, A_w_uv.reshape(Dc * H, D), A_w_o.reshape(H * D, M), B_w1, B_w2,
    ]
    out = pl.pallas_call(
        kernel,
        out_shape=jax.ShapeDtypeStruct((B, M), A_x.dtype),
        in_specs=[pl.BlockSpec(memory_space=pl.ANY)] * len(operands),
        scratch_shapes=[pltpu.VMEM(a.shape, a.dtype) for a in operands] + [
            pltpu.VMEM((max(M, Dc) * T, D), U32),
            pltpu.VMEM((Dc * T, D), U32),
            pltpu.VMEM((H, B, D), F32),
            pltpu.VMEM((c_tiles, H * B, _LANES), F32),
            pltpu.VMEM((B, H, Dc), BF16),
            pltpu.VMEM((B, T, H, keys), F32),
            pltpu.VMEM((c_tiles, B * H, _LANES), F32),
        ],
        compiler_params=pltpu.CompilerParams(vmem_limit_bytes=100 * 2**20),
    )(*operands)
    return out.reshape(A_x.shape)
```
